```python
import os as _os
_os.environ.setdefault("JAX_PLATFORMS", "cpu")
import jax
import jax.numpy as jnp

def _softmax(x, axis=-1):
    return jax.nn.softmax(x, axis=axis)
def _gelu(x):
    return jax.nn.gelu(x, approximate=True)
def _silu(x):
    return jax.nn.silu(x)
def _sigmoid(x):
    return jax.nn.sigmoid(x)
def _layernorm(x, axis=-1, eps=1e-5):
    m = jnp.mean(x, axis=axis, keepdims=True)
    v = jnp.var(x, axis=axis, keepdims=True)
    return (x - m) / jnp.sqrt(v + eps)
def _scatter_add(tgt, idx, src, axis=0):
    return tgt.at[idx].add(src)
def _segment_sum(src, seg, n):
    return jax.ops.segment_sum(src, seg, n)
class _Rng:
    def __init__(self, key):
        self._k = key
    def _next(self):
        self._k, sub = jax.random.split(self._k)
        return sub
    def normal(self, shape):
        return jax.random.normal(self._next(), shape, dtype=jnp.bfloat16)
    def randint(self, lo, hi, shape):
        return jax.random.randint(self._next(), shape, lo, hi, dtype=jnp.int32)
    def uniform(self, shape, lo=0.0, hi=1.0):
        return jax.random.uniform(self._next(), shape, jnp.bfloat16, lo, hi)
    def permutation(self, n):
        return jax.random.permutation(self._next(), n)


kernel_name = 'standalone__mha_softmax__decode'

def setup_inputs():
    _rng = _Rng(jax.random.key(int.from_bytes(__import__("os").urandom(4), "little")))
    _w = (lambda a: (lambda t: t.astype(jnp.bfloat16) if jnp.issubdtype(t.dtype, jnp.floating) else t)(jnp.asarray(a)))
    B, H, Sq, Sk, D = 1, 32, 1, 8192, 128
    return {
        "q": _w((lambda *s: _rng.normal(s) * 0.8)(B, H, Sq, D)),
        "k": _w((lambda *s: _rng.normal(s) * 0.8)(B, H, Sk, D)),
        "v": _w((lambda *s: _rng.normal(s) * 0.05)(B, H, Sk, D)),
    }

def reference(q, k, v):
    scale = q.shape[-1] ** -0.5
    scores = jnp.einsum("bhqd,bhkd->bhqk", q, k) * scale
    p = _softmax(scores, axis=-1)
    return jnp.einsum("bhqk,bhkd->bhqd", p, v)
```

```python
import functools
import math

import jax
import jax.numpy as jnp
from jax import lax
import jax.experimental.pallas as pl
import jax.experimental.pallas.tpu as pltpu

GROUP = 8
BLOCK = 128
SLAB = 16
SLABS = BLOCK // SLAB
SLOTS = 8
LOOK = SLOTS - 2


def _attention_kernel(
    q_hbm, k_hbm, v_hbm, o_hbm,
    q_buf, q_f32, k_buf, v_buf, m_ref, l_ref, acc_ref, o_buf,
    k_sem, v_sem, io_sem,
):
    heads, keys, dim = k_hbm.shape
    blocks = keys // BLOCK
    steps = (heads // GROUP) * blocks
    scale = dim ** -0.5 * math.log2(math.e)

    def group_rows(t):
        h0 = (t // blocks) * GROUP
        return pl.ds(h0 if isinstance(t, int) else pl.multiple_of(h0, GROUP), GROUP)

    def slab_copy(src, buf, sem, t, i):
        r0 = (t % blocks) * BLOCK + i * SLAB
        if not isinstance(t, int):
            r0 = pl.multiple_of(r0, SLAB)
        slot = t % SLOTS
        return pltpu.make_async_copy(
            src.at[group_rows(t), pl.ds(r0, SLAB)],
            buf.at[slot, :, pl.ds(i * SLAB, SLAB)],
            sem.at[slot * SLABS + i],
        )

    k_copy = functools.partial(slab_copy, k_hbm, k_buf, k_sem)
    v_copy = functools.partial(slab_copy, v_hbm, v_buf, v_sem)
    q_copy = pltpu.make_async_copy(q_hbm, q_buf, io_sem.at[0])
    o_copy = pltpu.make_async_copy(o_buf, o_hbm, io_sem.at[1])

    for i in range(SLABS):
        k_copy(0, i).start(priority=i % 2)
    q_copy.start()
    for t in range(LOOK):
        for i in range(SLABS):
            k_copy(t + 1, i).start(priority=0)
            v_copy(t, i).start(priority=1)

    m_ref[...] = jnp.full(m_ref.shape, -3.0e38, jnp.float32)
    l_ref[...] = jnp.zeros(l_ref.shape, jnp.float32)
    acc_ref[...] = jnp.zeros(acc_ref.shape, jnp.float32)
    q_copy.wait()
    q_f32[...] = q_buf[...].astype(jnp.float32)
    for i in range(SLABS):
        k_copy(0, i).wait()

    def per_head(matmul):
        out = matmul(0)
        head = lax.broadcasted_iota(jnp.int32, out.shape, 0)
        for h in range(1, GROUP):
            out = jnp.where(head == h, matmul(h), out)
        return out

    def probabilities(t):
        rows = group_rows(t)
        q = q_f32[rows].astype(k_buf.dtype)
        s = scale * per_head(lambda h: lax.dot_general(
            q, k_buf[t % SLOTS, h], (((1,), (1,)), ((), ())),
            preferred_element_type=jnp.float32))
        m_old = m_ref[rows]
        m_new = jnp.maximum(m_old, jnp.max(s, axis=-1, keepdims=True))
        alpha = jnp.exp2(m_old - m_new)
        p = jnp.exp2(s - m_new)
        m_ref[rows] = m_new
        l_ref[rows] = l_ref[rows] * alpha + p
        return p.astype(v_buf.dtype), alpha

    def accumulate(t, p, alpha):
        rows = group_rows(t)
        pv = per_head(lambda h: jnp.dot(
            p, v_buf[t % SLOTS, h], preferred_element_type=jnp.float32))
        acc_ref[rows] = acc_ref[rows] * alpha + pv

    def advance(t, wait_k, start_k, start_v):
        for i in range(SLABS):
            if wait_k:
                k_copy(t + 1, i).wait()
            v_copy(t, i).wait()
            if start_k:
                k_copy(t + 1 + LOOK, i).start(priority=0)
            if start_v:
                v_copy(t + LOOK, i).start(priority=1)

    def step(t, carry, *, wait_k=True, start_k=True, start_v=True):
        new_carry = probabilities(t)
        accumulate(t - 1, *carry)
        advance(t, wait_k, start_k, start_v)
        return new_carry

    carry = probabilities(0)
    advance(0, True, True, True)
    carry = lax.fori_loop(1, steps - 1 - LOOK, step, carry)
    carry = step(steps - 1 - LOOK, carry, start_k=False)
    carry = lax.fori_loop(
        steps - LOOK, steps - 1,
        functools.partial(step, start_k=False, start_v=False), carry)
    carry = step(steps - 1, carry, wait_k=False, start_k=False, start_v=False)
    accumulate(steps - 1, *carry)

    denominator = jnp.sum(l_ref[...], axis=-1, keepdims=True)
    o_buf[...] = (acc_ref[...] / denominator).astype(o_buf.dtype)
    o_copy.start()
    o_copy.wait()


@jax.jit
def pallas_standalone__mha_softmax__decode_kernel(
    q: jax.Array,
    k: jax.Array,
    v: jax.Array,
):
    batch, heads, q_len, dim = q.shape
    keys = k.shape[2]
    rows = batch * heads
    assert q_len == 1 and dim == BLOCK
    assert rows % GROUP == 0 and keys % BLOCK == 0

    ring = (SLOTS, GROUP, BLOCK, dim)
    out = pl.pallas_call(
        _attention_kernel,
        in_specs=[pl.BlockSpec(memory_space=pl.ANY)] * 3,
        out_specs=pl.BlockSpec(memory_space=pl.ANY),
        out_shape=jax.ShapeDtypeStruct((rows, dim), q.dtype),
        scratch_shapes=[
            pltpu.VMEM((rows, dim), q.dtype),
            pltpu.VMEM((rows, dim), jnp.float32),
            pltpu.VMEM(ring, k.dtype),
            pltpu.VMEM(ring, v.dtype),
            pltpu.VMEM((rows, BLOCK), jnp.float32),
            pltpu.VMEM((rows, BLOCK), jnp.float32),
            pltpu.VMEM((rows, dim), jnp.float32),
            pltpu.VMEM((rows, dim), q.dtype),
            pltpu.SemaphoreType.DMA((SLOTS * SLABS,)),
            pltpu.SemaphoreType.DMA((SLOTS * SLABS,)),
            pltpu.SemaphoreType.DMA((2,)),
        ],
        compiler_params=pltpu.CompilerParams(
            disable_bounds_checks=True, disable_semaphore_checks=True),
    )(q.reshape(rows, dim), k.reshape(rows, keys, dim), v.reshape(rows, keys, dim))
    return out.reshape(q.shape)
```

```python
import functools
import math

import jax
import jax.numpy as jnp
from jax import lax
import jax.experimental.pallas as pl
import jax.experimental.pallas.tpu as pltpu

SPLIT = 2
GROUP = 8
BLOCK = 128
COPY_ROWS = 64
GROUP_HEADS = GROUP // SPLIT
COPIES = GROUP_HEADS * (BLOCK // COPY_ROWS)
SLOTS = 8
K_LEAD = 32
V_LEAD = 38
SCORES_AFTER = 3
HIGH, LOW = 0, 1


def _attention_kernel(
    q_hbm, k_hbm, v_hbm, o_hbm,
    q_buf, q_seg, k_buf, v_buf, m_ref, l_ref, acc_ref,
    first_ref, factor_ref, late_ref, o_buf,
    k_sem, v_sem, io_sem,
):
    segments, segment_keys, dim = k_hbm.shape
    heads = segments // SPLIT
    blocks = segment_keys // BLOCK
    steps = (segments // GROUP) * blocks
    log_blocks = blocks.bit_length() - 1
    scale = dim ** -0.5 * math.log2(math.e)
    f32 = jnp.float32

    def aligned(x, n):
        return x if isinstance(x, int) else pl.multiple_of(x, n)

    def slot(t):
        return t & (SLOTS - 1)

    def group_rows(t):
        return pl.ds(aligned((t >> log_blocks) * GROUP, GROUP), GROUP)

    def block_copy(src, buf, sem, t, i):
        seg = (i % GROUP_HEADS) * SPLIT
        row = (i // GROUP_HEADS) * COPY_ROWS
        group = (t & (steps - 1)) >> log_blocks
        key = aligned((t & (blocks - 1)) * BLOCK + row, COPY_ROWS)
        return pltpu.make_async_copy(
            src.at[pl.ds(group * GROUP + seg, SPLIT), pl.ds(key, COPY_ROWS)],
            buf.at[slot(t), pl.ds(seg, SPLIT), pl.ds(row, COPY_ROWS)],
            sem,
        )

    def k_copy(t, i):
        return block_copy(k_hbm, k_buf, k_sem.at[slot(t)], t, i)

    def v_copy(t, i):
        return block_copy(v_hbm, v_buf, v_sem.at[slot(t) * COPIES + i], t, i)

    def wait_k_block(t):
        block = k_buf.at[slot(t)]
        pltpu.make_async_copy(block, block, k_sem.at[slot(t)]).wait()

    q_copy = pltpu.make_async_copy(q_hbm, q_buf, io_sem.at[0])
    o_copy = pltpu.make_async_copy(o_buf, o_hbm, io_sem.at[1])

    def fill_queues(t, _):
        for i in range(COPIES):
            n = t * COPIES + i
            pl.when(n < K_LEAD)(lambda: k_copy(t, i).start(priority=HIGH))
            pl.when(n < V_LEAD)(lambda: v_copy(t + 1, i).start(priority=LOW))
        pl.when(t == 0)(lambda: q_copy.start())

    lax.fori_loop(0, pl.cdiv(max(K_LEAD, V_LEAD), COPIES), fill_queues, None)

    m_ref[...] = jnp.full(m_ref.shape, -3.0e38, f32)
    l_ref[...] = jnp.zeros(l_ref.shape, f32)
    acc_ref[...] = jnp.zeros(acc_ref.shape, f32)
    q_copy.wait()
    for j in range(SPLIT):
        q_seg[pl.ds(j, heads, stride=SPLIT), :] = q_buf[...].astype(f32)

    sublane = lax.broadcasted_iota(jnp.int32, (GROUP, dim), 0)

    def tile(buf, t, s):
        return pltpu.bitcast(buf.bitcast(jnp.uint32)[slot(t), s], buf.dtype)

    def per_segment(matmul):
        out = matmul(0)
        for s in range(1, GROUP):
            out = jnp.where(sublane == s, matmul(s), out)
        return out

    def scores(t):
        q = q_seg[group_rows(t)].astype(k_buf.dtype)
        return scale * per_segment(lambda s: lax.dot_general(
            q, tile(k_buf, t, s), (((1,), (1,)), ((), ())),
            preferred_element_type=f32))

    def softmax(t, s):
        rows = group_rows(t)
        m_old = m_ref[rows]
        m_new = jnp.maximum(m_old, jnp.max(s, axis=-1, keepdims=True))
        alpha = jnp.exp2(m_old - m_new)
        p = jnp.exp2(s - m_new)
        m_ref[rows] = m_new
        l_ref[rows] = l_ref[rows] * alpha + p
        return p, alpha

    def accumulate(t, p, alpha):
        rows = group_rows(t)
        p = p.astype(v_buf.dtype)
        pv = per_segment(lambda s: jnp.dot(
            p, tile(v_buf, t, s), preferred_element_type=f32))
        acc_ref[rows] = acc_ref[rows] * alpha + pv

    def segment_rows(ref, j, n):
        return ref[pl.ds(j, n, stride=SPLIT), :]

    def merge_weights(n):
        m = [segment_rows(m_ref, j, n) for j in range(SPLIT)]
        m_head = functools.reduce(jnp.maximum, m)
        w = [jnp.exp2(x - m_head) for x in m]
        total = sum(segment_rows(l_ref, j, n) * w[j] for j in range(SPLIT))
        inverse = 1.0 / jnp.sum(total, axis=-1, keepdims=True)
        return [x * inverse for x in w]

    def prepare_late_block():
        for j, w in enumerate(merge_weights(GROUP)):
            factor_ref[pl.ds(j, GROUP, stride=SPLIT), :] = w
        rescale = jnp.exp2(first_ref[1] - m_ref[:GROUP]) * factor_ref[:GROUP]
        p = first_ref[0] * rescale
        diagonal = (lax.broadcasted_iota(jnp.int32, (BLOCK, BLOCK), 0)
                    == lax.broadcasted_iota(jnp.int32, (BLOCK, BLOCK), 1))
        ones = jnp.ones((BLOCK, dim), v_buf.dtype)
        for s in range(GROUP):
            spread = jnp.where(diagonal, p[s:s + 1], 0.0).astype(v_buf.dtype)
            late_ref[s] = jnp.dot(spread, ones, preferred_element_type=f32)

    def step(t, carry):
        for i in range(COPIES):
            v_copy(t, i).wait()
            if i == SCORES_AFTER:
                wait_k_block(t + 1)
            dk, ik = divmod(i + K_LEAD - COPIES, COPIES)
            dv, iv = divmod(i + V_LEAD, COPIES)
            pl.when(t + dk < steps)(
                lambda: k_copy(t + dk, ik).start(priority=HIGH))
            pl.when(t + dv <= steps)(
                lambda: v_copy(t + dv, iv).start(priority=LOW))
            if i == SCORES_AFTER:
                s = scores(t + 1)
        accumulate(t, *carry)
        carry = softmax(t + 1, s)
        pl.when(t == blocks)(prepare_late_block)
        return carry

    wait_k_block(0)
    first_ref[0], _ = softmax(0, scores(0))
    first_ref[1] = m_ref[:GROUP]
    wait_k_block(1)
    carry = lax.fori_loop(1, steps - 1, step, softmax(1, scores(1)))

    weights = merge_weights(heads)
    for i in range(COPIES):
        v_copy(steps - 1, i).wait()
    accumulate(steps - 1, *carry)
    out = sum(segment_rows(acc_ref, j, heads) * weights[j] for j in range(SPLIT))
    o_buf[...] = out.astype(o_buf.dtype)

    first = out[:GROUP]
    partial = [None] * GROUP_HEADS
    for i in range(COPIES):
        v_copy(steps, i).wait()
        head = i % GROUP_HEADS
        keys = pl.ds((i // GROUP_HEADS) * COPY_ROWS, COPY_ROWS)
        x = sum(v_buf[slot(steps), s, keys].astype(f32) * late_ref[s, keys]
                for s in range(head * SPLIT, (head + 1) * SPLIT))
        x = [x[r:r + GROUP] for r in range(0, COPY_ROWS, GROUP)]
        while len(x) > 1:
            x = [x[r] + x[r + 1] for r in range(0, len(x), 2)]
        partial[head] = x[0] if partial[head] is None else x[0] + partial[head]
        if i >= COPIES - GROUP_HEADS:
            total = jnp.sum(partial[head], axis=0, keepdims=True)
            first = jnp.where(sublane == head, first + total, first)
    o_buf[:GROUP] = first.astype(o_buf.dtype)
    o_copy.start()
    o_copy.wait()


@jax.jit
def pallas_standalone__mha_softmax__decode_kernel(
    q: jax.Array,
    k: jax.Array,
    v: jax.Array,
):
    batch, heads, q_len, dim = q.shape
    keys = k.shape[2]
    rows = batch * heads
    segments, segment_keys = rows * SPLIT, keys // SPLIT
    blocks = segment_keys // BLOCK
    steps = (segments // GROUP) * blocks
    assert q_len == 1 and dim == BLOCK and k.dtype.itemsize == v.dtype.itemsize == 2
    assert rows % GROUP == 0 and keys % (SPLIT * BLOCK) == 0
    assert blocks & (blocks - 1) == 0 and steps & (steps - 1) == 0
    assert blocks >= SLOTS

    ring = (SLOTS, GROUP, BLOCK, dim)
    state = pltpu.VMEM((segments, dim), jnp.float32)
    out = pl.pallas_call(
        _attention_kernel,
        in_specs=[pl.BlockSpec(memory_space=pl.ANY)] * 3,
        out_specs=pl.BlockSpec(memory_space=pl.ANY),
        out_shape=jax.ShapeDtypeStruct((rows, dim), q.dtype),
        scratch_shapes=[
            pltpu.VMEM((rows, dim), q.dtype),
            state,
            pltpu.VMEM(ring, k.dtype),
            pltpu.VMEM(ring, v.dtype),
            state,
            state,
            state,
            pltpu.VMEM((2, GROUP, BLOCK), jnp.float32),
            pltpu.VMEM((SPLIT * GROUP, dim), jnp.float32),
            pltpu.VMEM((GROUP, BLOCK, dim), jnp.float32),
            pltpu.VMEM((rows, dim), q.dtype),
            pltpu.SemaphoreType.DMA((SLOTS,)),
            pltpu.SemaphoreType.DMA((SLOTS * COPIES,)),
            pltpu.SemaphoreType.DMA((2,)),
        ],
        compiler_params=pltpu.CompilerParams(
            disable_bounds_checks=True, disable_semaphore_checks=True),
    )(
        q.reshape(rows, dim),
        k.reshape(segments, segment_keys, dim),
        v.reshape(segments, segment_keys, dim),
    )
    return out.reshape(q.shape)
```

```python
import functools
import math

import jax
import jax.numpy as jnp
from jax import lax
import jax.experimental.pallas as pl
import jax.experimental.pallas.tpu as pltpu

SPLIT = 2
GROUP = 8
BLOCK = 128
COPY_KEYS = 64
ROTATION = 64
GROUP_HEADS = GROUP // SPLIT
COPIES = GROUP_HEADS * (BLOCK // COPY_KEYS)
SLOTS = 8
HEAD_START = 24
K_LEAD = 4
V_AHEAD = 14
HIGH, LOW = 0, 1


def _attention_kernel(
    q_hbm, k_hbm, v_hbm, o_hbm,
    q_buf, q_seg, k_buf, v_buf, m_ref, l_ref, acc_ref,
    v_late, p_late, m_late, w_late, factor_ref, o_buf,
    k_sem, v_sem, late_sem, o_sem,
):
    segments, segment_keys, dim = k_hbm.shape
    heads = segments // SPLIT
    blocks = segment_keys // BLOCK
    steps = (segments // GROUP) * blocks
    log_blocks = blocks.bit_length() - 1
    scale = dim ** -0.5 * math.log2(math.e)
    f32 = jnp.float32

    def aligned(x, n):
        return x if isinstance(x, int) else pl.multiple_of(x, n)

    def slot(t):
        return t & (SLOTS - 1)

    def group_rows(t):
        return pl.ds(aligned((t >> log_blocks) * GROUP, GROUP), GROUP)

    def block_copy(src, dst, sem, t, i):
        seg = (i % GROUP_HEADS) * SPLIT
        row = (i // GROUP_HEADS) * COPY_KEYS
        key = (t * BLOCK + row + ROTATION) & (segment_keys - 1)
        return pltpu.make_async_copy(
            src.at[pl.ds((t >> log_blocks) * GROUP + seg, SPLIT),
                   pl.ds(aligned(key, COPY_KEYS), COPY_KEYS)],
            dst.at[pl.ds(seg, SPLIT), pl.ds(row, COPY_KEYS)],
            sem,
        )

    def ring_copy(src, buf, sem, t, n):
        t, i = t + n // COPIES, n % COPIES
        return block_copy(src, buf.at[slot(t)], sem.at[slot(t)], t, i)

    def wait_block(buf, sem, t):
        block = buf.at[slot(t)]
        pltpu.make_async_copy(block, block, sem.at[slot(t)]).wait()

    def late_copy(i):
        return block_copy(v_hbm, v_late, late_sem.at[i], 0, i)

    k_copy = functools.partial(ring_copy, k_hbm, k_buf, k_sem)
    v_copy = functools.partial(ring_copy, v_hbm, v_buf, v_sem)
    wait_k = functools.partial(wait_block, k_buf, k_sem)
    wait_v = functools.partial(wait_block, v_buf, v_sem)

    q_copy = pltpu.make_async_copy(q_hbm, q_buf, k_sem.at[SLOTS])
    q_copy.start()
    first_in_loop = (1 + K_LEAD) * COPIES
    high = [k_copy(0, n) for n in range(0, HEAD_START, 2)]
    high += [k_copy(0, n) for n in range(HEAD_START, first_in_loop)]
    low = [k_copy(0, n) for n in range(1, HEAD_START, 2)]
    low += [v_copy(0, n) for n in range(COPIES, first_in_loop + V_AHEAD)]
    backlog = len(low) - len(high)
    for copy in low[:backlog]:
        copy.start(priority=LOW)
    for high_copy, low_copy in zip(high, low[backlog:]):
        high_copy.start(priority=HIGH)
        low_copy.start(priority=LOW)

    m_ref[...] = jnp.full(m_ref.shape, -3.0e38, f32)
    l_ref[...] = jnp.zeros(l_ref.shape, f32)
    acc_ref[...] = jnp.zeros(acc_ref.shape, f32)
    q_copy.wait()
    for j in range(SPLIT):
        q_seg[pl.ds(j, heads, stride=SPLIT), :] = q_buf[...].astype(f32)

    sublane = lax.broadcasted_iota(jnp.int32, (GROUP, dim), 0)

    def tile(buf, t, s):
        return pltpu.bitcast(buf.bitcast(jnp.uint32)[slot(t), s], buf.dtype)

    def per_segment(matmul):
        out = matmul(0)
        for s in range(1, GROUP):
            out = jnp.where(sublane == s, matmul(s), out)
        return out

    def probabilities(t):
        rows = group_rows(t)
        q = q_seg[rows].astype(k_buf.dtype)
        scores = scale * per_segment(lambda s: lax.dot_general(
            q, tile(k_buf, t, s), (((1,), (1,)), ((), ())),
            preferred_element_type=f32))
        m_old = m_ref[rows]
        m_new = jnp.maximum(m_old, jnp.max(scores, axis=-1, keepdims=True))
        alpha = jnp.exp2(m_old - m_new)
        p = jnp.exp2(scores - m_new)
        m_ref[rows] = m_new
        l_ref[rows] = l_ref[rows] * alpha + p
        return p, alpha

    def accumulate(t, p, alpha):
        rows = group_rows(t)
        p = p.astype(v_buf.dtype)
        pv = per_segment(lambda s: jnp.dot(
            p, tile(v_buf, t, s), preferred_element_type=f32))
        acc_ref[rows] = acc_ref[rows] * alpha + pv

    def segment_rows(ref, j, n):
        return ref[pl.ds(j, n, stride=SPLIT), :]

    def merge_weights(n):
        m = [segment_rows(m_ref, j, n) for j in range(SPLIT)]
        m_head = functools.reduce(jnp.maximum, m)
        w = [jnp.exp2(x - m_head) for x in m]
        total = sum(segment_rows(l_ref, j, n) * w[j] for j in range(SPLIT))
        inverse = 1.0 / jnp.sum(total, axis=-1, keepdims=True)
        return [x * inverse for x in w]

    def prepare_late_block():
        for j, w in enumerate(merge_weights(GROUP)):
            factor_ref[pl.ds(j, GROUP, stride=SPLIT), :] = w
        rescale = jnp.exp2(m_late[...] - m_ref[:GROUP]) * factor_ref[:GROUP]
        p = p_late[...] * rescale
        diagonal = (lax.broadcasted_iota(jnp.int32, (BLOCK, BLOCK), 0)
                    == lax.broadcasted_iota(jnp.int32, (BLOCK, BLOCK), 1))
        ones = jnp.ones((BLOCK, dim), v_buf.dtype)
        for s in range(GROUP):
            spread = jnp.where(diagonal, p[s:s + 1], 0.0).astype(v_buf.dtype)
            w_late[s] = jnp.dot(spread, ones, preferred_element_type=f32)

    def step(t, carry):
        wait_k(t + 1)
        next_carry = probabilities(t + 1)
        accumulate(t, *carry)
        return next_carry

    def streaming_step(t, carry):
        wait_v(t)
        for i in range(COPIES):
            k_copy(t + K_LEAD, i).start(priority=HIGH)
            v_copy(t + K_LEAD, i + V_AHEAD).start(priority=LOW)
        carry = step(t, carry)
        pl.when(t == blocks)(prepare_late_block)
        return carry

    def draining_step(t, carry):
        wait_v(t)
        return step(t, carry)

    wait_k(0)
    p_late[...], _ = probabilities(0)
    m_late[...] = m_ref[:GROUP]
    wait_k(1)
    last_blocks = pl.cdiv(V_AHEAD, COPIES)
    drain = steps - K_LEAD - last_blocks
    carry = lax.fori_loop(1, drain, streaming_step, probabilities(1))

    t = steps - last_blocks
    high = [k_copy(t, n) for n in range(last_blocks * COPIES)]
    low = [v_copy(t, n) for n in range(V_AHEAD, last_blocks * COPIES)]
    low += [late_copy(i) for i in range(COPIES)]
    for n, high_copy in enumerate(high):
        high_copy.start(priority=HIGH)
        if n < len(low):
            low[n].start(priority=LOW)
    carry = lax.fori_loop(drain, steps - 1, draining_step, carry)

    wait_v(steps - 1)
    weights = merge_weights(heads)
    accumulate(steps - 1, *carry)
    out = sum(segment_rows(acc_ref, j, heads) * weights[j] for j in range(SPLIT))
    o_buf[...] = out.astype(o_buf.dtype)

    def output_copy(rows, sem):
        return pltpu.make_async_copy(o_buf.at[rows], o_hbm.at[rows], sem)

    rest_copy = output_copy(pl.ds(GROUP, heads - GROUP), o_sem.at[0])
    first_copy = output_copy(pl.ds(0, GROUP), o_sem.at[1])
    first = out[:GROUP]
    partial = [None] * GROUP_HEADS
    for i in range(COPIES):
        if i == COPIES - 1:
            rest_copy.start()
        late_copy(i).wait()
        head = i % GROUP_HEADS
        keys = pl.ds((i // GROUP_HEADS) * COPY_KEYS, COPY_KEYS)
        x = sum(v_late[s, keys].astype(f32) * w_late[s, keys]
                for s in range(head * SPLIT, (head + 1) * SPLIT))
        x = [x[r:r + GROUP] for r in range(0, COPY_KEYS, GROUP)]
        while len(x) > 1:
            x = [x[r] + x[r + 1] for r in range(0, len(x), 2)]
        partial[head] = x[0] if partial[head] is None else x[0] + partial[head]
        if i >= COPIES - 2:
            for done in [head] if i == COPIES - 1 else range(head + 1):
                total = jnp.sum(partial[done], axis=0, keepdims=True)
                first = jnp.where(sublane == done, first + total, first)
    o_buf[:GROUP] = first.astype(o_buf.dtype)
    first_copy.start()
    rest_copy.wait()
    first_copy.wait()


@jax.jit
def pallas_standalone__mha_softmax__decode_kernel(
    q: jax.Array,
    k: jax.Array,
    v: jax.Array,
):
    batch, heads, q_len, dim = q.shape
    keys = k.shape[2]
    rows = batch * heads
    segments, segment_keys = rows * SPLIT, keys // SPLIT
    assert q_len == 1 and dim == BLOCK
    assert k.dtype.itemsize == v.dtype.itemsize == 2
    assert rows % GROUP == 0 and rows > GROUP
    assert keys & (keys - 1) == 0 and segment_keys >= SLOTS * BLOCK

    block = (GROUP, BLOCK, dim)
    state = pltpu.VMEM((segments, dim), jnp.float32)
    out = pl.pallas_call(
        _attention_kernel,
        in_specs=[pl.BlockSpec(memory_space=pl.ANY)] * 3,
        out_specs=pl.BlockSpec(memory_space=pl.ANY),
        out_shape=jax.ShapeDtypeStruct((rows, dim), q.dtype),
        scratch_shapes=[
            pltpu.VMEM((rows, dim), q.dtype),
            state,
            pltpu.VMEM((SLOTS, *block), k.dtype),
            pltpu.VMEM((SLOTS, *block), v.dtype),
            state,
            state,
            state,
            pltpu.VMEM(block, v.dtype),
            pltpu.VMEM((GROUP, BLOCK), jnp.float32),
            pltpu.VMEM((GROUP, BLOCK), jnp.float32),
            pltpu.VMEM(block, jnp.float32),
            pltpu.VMEM((SPLIT * GROUP, dim), jnp.float32),
            pltpu.VMEM((rows, dim), q.dtype),
            pltpu.SemaphoreType.DMA((SLOTS + 1,)),
            pltpu.SemaphoreType.DMA((SLOTS,)),
            pltpu.SemaphoreType.DMA((COPIES,)),
            pltpu.SemaphoreType.DMA((2,)),
        ],
        compiler_params=pltpu.CompilerParams(
            disable_bounds_checks=True, disable_semaphore_checks=True),
    )(
        q.reshape(rows, dim),
        k.reshape(segments, segment_keys, dim),
        v.reshape(segments, segment_keys, dim),
    )
    return out.reshape(q.shape)
```

```python
import functools
import math

import jax
import jax.numpy as jnp
from jax import lax
import jax.experimental.pallas as pl
import jax.experimental.pallas.tpu as pltpu

SPLIT = 2
GROUP = 8
BLOCK = 128
COPY_KEYS = 64
ROTATION = 64
GROUP_HEADS = GROUP // SPLIT
COPIES = GROUP_HEADS * (BLOCK // COPY_KEYS)
SLOTS = 8
HEAD_START = 24
K_LEAD = 4
V_AHEAD = 14
HIGH, LOW = 0, 1


def _attention_kernel(
    q_hbm, k_hbm, v_hbm, o_hbm,
    q_buf, q_seg, k_buf, v_buf, m_ref, l_ref, acc_ref,
    p_late, m_late, w_late, factor_ref, o_buf,
    k_sem, v_sem, o_sem,
):
    segments, segment_keys, dim = k_hbm.shape
    heads = segments // SPLIT
    blocks = segment_keys // BLOCK
    steps = (segments // GROUP) * blocks
    log_blocks = blocks.bit_length() - 1
    scale = dim ** -0.5 * math.log2(math.e)
    f32 = jnp.float32

    def aligned(x, n):
        return x if isinstance(x, int) else pl.multiple_of(x, n)

    def slot(t):
        return t & (SLOTS - 1)

    def group_rows(t):
        return pl.ds(aligned((t >> log_blocks) * GROUP, GROUP), GROUP)

    def block_copy(src, dst, sem, t, i):
        seg = (i % GROUP_HEADS) * SPLIT
        row = (i // GROUP_HEADS) * COPY_KEYS
        key = (t * BLOCK + row + ROTATION) & (segment_keys - 1)
        return pltpu.make_async_copy(
            src.at[pl.ds((t >> log_blocks) * GROUP + seg, SPLIT),
                   pl.ds(aligned(key, COPY_KEYS), COPY_KEYS)],
            dst.at[pl.ds(seg, SPLIT), pl.ds(row, COPY_KEYS)],
            sem,
        )

    def ring_copy(src, buf, sem, t, n):
        t, i = t + n // COPIES, n % COPIES
        return block_copy(src, buf.at[slot(t)], sem.at[slot(t)], t, i)

    def wait_block(buf, sem, t):
        block = buf.at[slot(t)]
        pltpu.make_async_copy(block, block, sem.at[slot(t)]).wait()

    v_late = v_buf.at[slot(steps)]

    def late_copy(i):
        return block_copy(v_hbm, v_late, v_sem.at[SLOTS + i], 0, i)

    k_copy = functools.partial(ring_copy, k_hbm, k_buf, k_sem)
    v_copy = functools.partial(ring_copy, v_hbm, v_buf, v_sem)
    wait_k = functools.partial(wait_block, k_buf, k_sem)
    wait_v = functools.partial(wait_block, v_buf, v_sem)

    q_copy = pltpu.make_async_copy(q_hbm, q_buf, k_sem.at[SLOTS])
    q_copy.start()
    first_in_loop = (1 + K_LEAD) * COPIES
    high = [k_copy(0, n) for n in range(0, HEAD_START, 2)]
    high += [k_copy(0, n) for n in range(HEAD_START, first_in_loop)]
    low = [k_copy(0, n) for n in range(1, HEAD_START, 2)]
    low += [v_copy(0, n) for n in range(COPIES, first_in_loop + V_AHEAD)]
    backlog = len(low) - len(high)
    for copy in low[:backlog]:
        copy.start(priority=LOW)
    for high_copy, low_copy in zip(high, low[backlog:]):
        high_copy.start(priority=HIGH)
        low_copy.start(priority=LOW)

    m_ref[...] = jnp.full(m_ref.shape, -3.0e38, f32)
    l_ref[...] = jnp.zeros(l_ref.shape, f32)
    acc_ref[...] = jnp.zeros(acc_ref.shape, f32)
    q_copy.wait()
    for j in range(SPLIT):
        q_seg[pl.ds(j, heads, stride=SPLIT), :] = q_buf[...].astype(f32)

    sublane = lax.broadcasted_iota(jnp.int32, (GROUP, dim), 0)

    def tile(buf, t, s):
        return pltpu.bitcast(buf.bitcast(jnp.uint32)[slot(t), s], buf.dtype)

    def per_segment(matmul):
        out = matmul(0)
        for s in range(1, GROUP):
            out = jnp.where(sublane == s, matmul(s), out)
        return out

    def probabilities(t):
        rows = group_rows(t)
        q = q_seg[rows].astype(k_buf.dtype)
        scores = scale * per_segment(lambda s: lax.dot_general(
            q, tile(k_buf, t, s), (((1,), (1,)), ((), ())),
            preferred_element_type=f32))
        m_old = m_ref[rows]
        m_new = jnp.maximum(m_old, jnp.max(scores, axis=-1, keepdims=True))
        alpha = jnp.exp2(m_old - m_new)
        p = jnp.exp2(scores - m_new)
        m_ref[rows] = m_new
        l_ref[rows] = l_ref[rows] * alpha + p
        return p, alpha

    def accumulate(t, p, alpha):
        rows = group_rows(t)
        p = p.astype(v_buf.dtype)
        pv = per_segment(lambda s: jnp.dot(
            p, tile(v_buf, t, s), preferred_element_type=f32))
        acc_ref[rows] = acc_ref[rows] * alpha + pv

    def segment_rows(ref, j, n):
        return ref[pl.ds(j, n, stride=SPLIT), :]

    def merge_weights(n):
        m = [segment_rows(m_ref, j, n) for j in range(SPLIT)]
        m_head = functools.reduce(jnp.maximum, m)
        w = [jnp.exp2(x - m_head) for x in m]
        total = sum(segment_rows(l_ref, j, n) * w[j] for j in range(SPLIT))
        inverse = 1.0 / jnp.sum(total, axis=-1, keepdims=True)
        return [x * inverse for x in w]

    def prepare_late_block():
        for j, w in enumerate(merge_weights(GROUP)):
            factor_ref[pl.ds(j, GROUP, stride=SPLIT), :] = w
        rescale = jnp.exp2(m_late[...] - m_ref[:GROUP]) * factor_ref[:GROUP]
        p = p_late[...] * rescale
        diagonal = (lax.broadcasted_iota(jnp.int32, (BLOCK, BLOCK), 0)
                    == lax.broadcasted_iota(jnp.int32, (BLOCK, BLOCK), 1))
        ones = jnp.ones((BLOCK, dim), v_buf.dtype)
        for s in range(GROUP):
            spread = jnp.where(diagonal, p[s:s + 1], 0.0).astype(v_buf.dtype)
            w_late[s] = jnp.dot(spread, ones, preferred_element_type=f32)

    def step(t, carry):
        wait_k(t + 1)
        next_carry = probabilities(t + 1)
        accumulate(t, *carry)
        return next_carry

    def streaming_step(t, carry):
        wait_v(t)
        for i in range(COPIES):
            k_copy(t + K_LEAD, i).start(priority=HIGH)
            v_copy(t + K_LEAD, i + V_AHEAD).start(priority=LOW)
        carry = step(t, carry)
        pl.when(t == blocks)(prepare_late_block)
        return carry

    def draining_step(t, carry):
        wait_v(t)
        return step(t, carry)

    wait_k(0)
    p_late[...], _ = probabilities(0)
    m_late[...] = m_ref[:GROUP]
    wait_k(1)
    last_blocks = pl.cdiv(V_AHEAD, COPIES)
    drain = steps - K_LEAD - last_blocks
    carry = lax.fori_loop(1, drain, streaming_step, probabilities(1))

    t = steps - last_blocks
    high = [k_copy(t, n) for n in range(last_blocks * COPIES)]
    low = [v_copy(t, n) for n in range(V_AHEAD, last_blocks * COPIES)]
    low += [late_copy(i) for i in range(COPIES)]
    for n, high_copy in enumerate(high):
        high_copy.start(priority=HIGH)
        if n < len(low):
            low[n].start(priority=LOW)
    carry = lax.fori_loop(drain, steps - 1, draining_step, carry)

    wait_v(steps - 1)
    weights = merge_weights(heads)
    accumulate(steps - 1, *carry)
    out = sum(segment_rows(acc_ref, j, heads) * weights[j] for j in range(SPLIT))
    o_buf[...] = out.astype(o_buf.dtype)

    def output_copy(rows, sem):
        return pltpu.make_async_copy(o_buf.at[rows], o_hbm.at[rows], sem)

    rest_copy = output_copy(pl.ds(GROUP, heads - GROUP), o_sem.at[0])
    first_copy = output_copy(pl.ds(0, GROUP), o_sem.at[1])
    first = out[:GROUP]
    partial = [None] * GROUP_HEADS
    for i in range(COPIES):
        if i == COPIES - 1:
            rest_copy.start()
        late_copy(i).wait()
        head = i % GROUP_HEADS
        keys = pl.ds((i // GROUP_HEADS) * COPY_KEYS, COPY_KEYS)
        x = sum(v_late[s, keys].astype(f32) * w_late[s, keys]
                for s in range(head * SPLIT, (head + 1) * SPLIT))
        x = [x[r:r + GROUP] for r in range(0, COPY_KEYS, GROUP)]
        while len(x) > 1:
            x = [x[r] + x[r + 1] for r in range(0, len(x), 2)]
        partial[head] = x[0] if partial[head] is None else x[0] + partial[head]
        if i >= COPIES - 2:
            for done in [head] if i == COPIES - 1 else range(head + 1):
                total = jnp.sum(partial[done], axis=0, keepdims=True)
                first = jnp.where(sublane == done, first + total, first)
    o_buf[:GROUP] = first.astype(o_buf.dtype)
    first_copy.start()
    rest_copy.wait()
    first_copy.wait()


@jax.jit
def pallas_standalone__mha_softmax__decode_kernel(
    q: jax.Array,
    k: jax.Array,
    v: jax.Array,
):
    batch, heads, q_len, dim = q.shape
    keys = k.shape[2]
    rows = batch * heads
    segments, segment_keys = rows * SPLIT, keys // SPLIT
    assert q_len == 1 and dim == BLOCK
    assert k.dtype.itemsize == v.dtype.itemsize == 2
    assert rows % GROUP == 0 and rows > GROUP
    assert keys & (keys - 1) == 0 and segment_keys >= SLOTS * BLOCK

    block = (GROUP, BLOCK, dim)
    state = pltpu.VMEM((segments, dim), jnp.float32)
    out = pl.pallas_call(
        _attention_kernel,
        in_specs=[pl.BlockSpec(memory_space=pl.ANY)] * 3,
        out_specs=pl.BlockSpec(memory_space=pl.ANY),
        out_shape=jax.ShapeDtypeStruct((rows, dim), q.dtype),
        scratch_shapes=[
            pltpu.VMEM((rows, dim), q.dtype),
            state,
            pltpu.VMEM((SLOTS, *block), k.dtype),
            pltpu.VMEM((SLOTS, *block), v.dtype),
            state,
            state,
            state,
            pltpu.VMEM((GROUP, BLOCK), jnp.float32),
            pltpu.VMEM((GROUP, BLOCK), jnp.float32),
            pltpu.VMEM(block, jnp.float32),
            pltpu.VMEM((SPLIT * GROUP, dim), jnp.float32),
            pltpu.VMEM((rows, dim), q.dtype),
            pltpu.SemaphoreType.DMA((SLOTS + 1,)),
            pltpu.SemaphoreType.DMA((SLOTS + COPIES,)),
            pltpu.SemaphoreType.DMA((2,)),
        ],
        compiler_params=pltpu.CompilerParams(
            disable_bounds_checks=True, disable_semaphore_checks=True),
    )(
        q.reshape(rows, dim),
        k.reshape(segments, segment_keys, dim),
        v.reshape(segments, segment_keys, dim),
    )
    return out.reshape(q.shape)
```

```python
import functools
import math

import jax
import jax.numpy as jnp
from jax import lax
import jax.experimental.pallas as pl
import jax.experimental.pallas.tpu as pltpu
import numpy as np

GROUP = 8
GROUP_HEADS = GROUP // 2
BLOCK = 128
COPY_KEYS = 64
ROTATION = 64
COPIES = GROUP_HEADS * (BLOCK // COPY_KEYS)
SLOTS = 8
HEAD_START = 22
K_LEAD = 4
V_AHEAD = 14
HIGH, LOW = 0, 1

K_SEM, V_SEM, LATE_SEM, Q_SEM = 0, SLOTS, 2 * SLOTS, 2 * SLOTS + COPIES


def _attention_kernel(
    q_hbm, k_hbm, v_hbm, o_hbm,
    q_buf, q_seg, k_buf, v_buf, m_ref, l_ref, acc_ref,
    v_late, p_late, m_late, w_late, o_first, o_rest,
    sem, o_sem,
):
    segments, segment_keys, dim = k_hbm.shape
    groups = segments // GROUP
    blocks = segment_keys // BLOCK
    steps = groups * blocks
    log_blocks = blocks.bit_length() - 1
    scale = dim ** -0.5 * math.log2(math.e)
    f32 = jnp.float32

    def aligned(x, n):
        return x if isinstance(x, int) else pl.multiple_of(x, n)

    def slot(t):
        return t & (SLOTS - 1)

    def block_copy(src, dst, dma_sem, t, i):
        seg = (i % GROUP_HEADS) * 2
        row = (i // GROUP_HEADS) * COPY_KEYS
        key = (t * BLOCK + row + ROTATION) & (segment_keys - 1)
        return pltpu.make_async_copy(
            src.at[pl.ds((t >> log_blocks) * GROUP + seg, 2),
                   pl.ds(aligned(key, COPY_KEYS), COPY_KEYS)],
            dst.at[pl.ds(seg, 2), pl.ds(row, COPY_KEYS)],
            dma_sem,
        )

    def ring_copy(src, buf, first_sem, t, n):
        t, i = t + n // COPIES, n % COPIES
        return block_copy(src, buf.at[slot(t)], sem.at[first_sem + slot(t)], t, i)

    def wait_block(buf, first_sem, t):
        block = buf.at[slot(t)]
        pltpu.make_async_copy(block, block, sem.at[first_sem + slot(t)]).wait()

    def late_copy(i):
        return block_copy(v_hbm, v_late, sem.at[LATE_SEM + i], 0, i)

    k_copy = functools.partial(ring_copy, k_hbm, k_buf, K_SEM)
    v_copy = functools.partial(ring_copy, v_hbm, v_buf, V_SEM)
    wait_k = functools.partial(wait_block, k_buf, K_SEM)
    wait_v = functools.partial(wait_block, v_buf, V_SEM)
    q_copy = pltpu.make_async_copy(q_hbm, q_buf, sem.at[Q_SEM])

    first_in_loop = (1 + K_LEAD) * COPIES
    high = [k_copy(0, n) for n in range(0, HEAD_START, 2)]
    high += [k_copy(0, n) for n in range(HEAD_START, first_in_loop)]
    low = [k_copy(0, n) for n in range(1, HEAD_START, 2)]
    low += [v_copy(0, n) for n in range(COPIES, first_in_loop + V_AHEAD)]
    backlog = len(low) - len(high)
    for n, copy in enumerate(low[:backlog]):
        copy.start(priority=LOW)
        if n == 3:
            q_copy.start(priority=HIGH)
    for high_copy, low_copy in zip(high, low[backlog:]):
        high_copy.start(priority=HIGH)
        low_copy.start(priority=LOW)

    sublane = lax.broadcasted_iota(jnp.int32, (GROUP, dim), 0)

    def swap_halves(x):
        return jnp.concatenate([x[GROUP_HEADS:], x[:GROUP_HEADS]], axis=0)

    m_ref[...] = jnp.full(m_ref.shape, np.finfo(np.float32).min, f32)
    l_ref[...] = jnp.zeros(l_ref.shape, f32)
    acc_ref[...] = jnp.zeros(acc_ref.shape, f32)
    q_copy.wait()
    q = q_buf[...].astype(f32)
    for g in range(groups):
        q_group = q[g * GROUP_HEADS:(g + 1) * GROUP_HEADS]
        q_seg[g] = jnp.concatenate([q_group, q_group], axis=0)

    def tile(s):
        return (s % GROUP_HEADS) * 2 + s // GROUP_HEADS

    def per_segment(matmul):
        out = matmul(tile(0))
        for s in range(1, GROUP):
            out = jnp.where(sublane == s, matmul(tile(s)), out)
        return out

    def probabilities(t):
        g = t >> log_blocks
        q_group = q_seg[g].astype(k_buf.dtype)
        scores = scale * per_segment(lambda j: lax.dot_general(
            q_group, k_buf[slot(t), j], (((1,), (1,)), ((), ())),
            preferred_element_type=f32))
        m_old = m_ref[g]
        m_new = jnp.maximum(m_old, jnp.max(scores, axis=-1, keepdims=True))
        alpha = jnp.exp2(m_old - m_new)
        p = jnp.exp2(scores - m_new)
        m_ref[g] = m_new
        l_ref[g] = l_ref[g] * alpha + p
        return p, alpha

    def accumulate(t, p, alpha):
        g = t >> log_blocks
        p = p.astype(v_buf.dtype)
        pv = per_segment(lambda j: jnp.dot(
            p, v_buf[slot(t), j], preferred_element_type=f32))
        acc_ref[g] = acc_ref[g] * alpha + pv

    def merge_weight(g):
        m = m_ref[g]
        w = jnp.exp2(m - jnp.maximum(m, swap_halves(m)))
        total = l_ref[g] * w
        return w / jnp.sum(total + swap_halves(total), axis=-1, keepdims=True)

    def prepare_late_block():
        rescale = jnp.exp2(m_late[...] - m_ref[0]) * merge_weight(0)
        p = p_late[...] * rescale
        diagonal = (lax.broadcasted_iota(jnp.int32, (BLOCK, BLOCK), 0)
                    == lax.broadcasted_iota(jnp.int32, (BLOCK, BLOCK), 1))
        ones = jnp.ones((BLOCK, dim), v_buf.dtype)
        for s in range(GROUP):
            spread = jnp.where(diagonal, p[s:s + 1], 0.0).astype(v_buf.dtype)
            w_late[tile(s)] = jnp.dot(spread, ones, preferred_element_type=f32)

    def step(t, carry):
        wait_k(t + 1)
        next_carry = probabilities(t + 1)
        accumulate(t, *carry)
        return next_carry

    def streaming_step(t, carry):
        wait_v(t)
        for i in range(COPIES):
            k_copy(t + K_LEAD, i).start(priority=HIGH)
            v_copy(t + K_LEAD, i + V_AHEAD).start(priority=LOW)
        carry = step(t, carry)
        pl.when(t == blocks)(prepare_late_block)
        return carry

    def draining_step(t, carry):
        wait_v(t)
        return step(t, carry)

    wait_k(0)
    p_late[...], _ = probabilities(0)
    m_late[...] = m_ref[0]
    wait_k(1)
    last_blocks = pl.cdiv(V_AHEAD, COPIES)
    drain = steps - K_LEAD - last_blocks
    carry = lax.fori_loop(1, drain, streaming_step, probabilities(1))

    t = steps - last_blocks
    high = [k_copy(t, n) for n in range(last_blocks * COPIES)]
    low = [v_copy(t, n) for n in range(V_AHEAD, last_blocks * COPIES)]
    low += [late_copy(i) for i in range(COPIES)]
    for n in range(max(len(high), len(low))):
        if n < len(high):
            high[n].start(priority=HIGH)
        if n < len(low):
            low[n].start(priority=LOW)
    carry = lax.fori_loop(drain, steps - 1, draining_step, carry)

    wait_v(steps - 1)
    accumulate(steps - 1, *carry)
    out = []
    for g in range(groups):
        x = acc_ref[g] * merge_weight(g)
        out.append(x + swap_halves(x))
    out = [jnp.where(sublane < GROUP_HEADS, out[g], out[g + 1])
           for g in range(0, groups, 2)]
    o_rest[...] = jnp.concatenate(out[1:], axis=0).astype(o_rest.dtype)

    first_copy = pltpu.make_async_copy(
        o_first, o_hbm.at[pl.ds(0, GROUP)], o_sem.at[0])
    rest_copy = pltpu.make_async_copy(
        o_rest, o_hbm.at[pl.ds(GROUP, o_rest.shape[0])], o_sem.at[1])
    first = out[0]
    partial = [None] * GROUP_HEADS
    for i in range(COPIES):
        if i == COPIES - 1:
            rest_copy.start()
        late_copy(i).wait()
        head = i % GROUP_HEADS
        keys = pl.ds((i // GROUP_HEADS) * COPY_KEYS, COPY_KEYS)
        x = sum(v_late[j, keys].astype(f32) * w_late[j, keys]
                for j in (2 * head, 2 * head + 1))
        x = [x[r:r + GROUP] for r in range(0, COPY_KEYS, GROUP)]
        while len(x) > 1:
            x = [x[r] + x[r + 1] for r in range(0, len(x), 2)]
        partial[head] = x[0] if partial[head] is None else x[0] + partial[head]
        if i >= COPIES - 2:
            for done in [head] if i == COPIES - 1 else range(head + 1):
                total = jnp.sum(partial[done], axis=0, keepdims=True)
                first = jnp.where(sublane == done, first + total, first)
    o_first[...] = first.astype(o_first.dtype)
    first_copy.start()
    rest_copy.wait()
    first_copy.wait()


@jax.jit
def pallas_standalone__mha_softmax__decode_kernel(
    q: jax.Array,
    k: jax.Array,
    v: jax.Array,
):
    batch, heads, q_len, dim = q.shape
    keys = k.shape[2]
    rows = batch * heads
    segments, segment_keys = 2 * rows, keys // 2
    assert q_len == 1 and dim == BLOCK
    assert rows % GROUP == 0 and rows > GROUP
    assert keys & (keys - 1) == 0 and segment_keys >= SLOTS * BLOCK

    block = (GROUP, BLOCK, dim)
    state = pltpu.VMEM((segments // GROUP, GROUP, dim), jnp.float32)
    out = pl.pallas_call(
        _attention_kernel,
        in_specs=[pl.BlockSpec(memory_space=pl.ANY)] * 3,
        out_specs=pl.BlockSpec(memory_space=pl.ANY),
        out_shape=jax.ShapeDtypeStruct((rows, dim), q.dtype),
        scratch_shapes=[
            pltpu.VMEM((rows, dim), q.dtype),
            state,
            pltpu.VMEM((SLOTS, *block), k.dtype),
            pltpu.VMEM((SLOTS, *block), v.dtype),
            state,
            state,
            state,
            pltpu.VMEM(block, v.dtype),
            pltpu.VMEM((GROUP, BLOCK), jnp.float32),
            pltpu.VMEM((GROUP, BLOCK), jnp.float32),
            pltpu.VMEM(block, jnp.float32),
            pltpu.VMEM((GROUP, dim), q.dtype),
            pltpu.VMEM((rows - GROUP, dim), q.dtype),
            pltpu.SemaphoreType.DMA((Q_SEM + 1,)),
            pltpu.SemaphoreType.DMA((2,)),
        ],
        compiler_params=pltpu.CompilerParams(disable_semaphore_checks=True),
    )(
        q.reshape(rows, dim),
        k.reshape(segments, segment_keys, dim),
        v.reshape(segments, segment_keys, dim),
    )
    return out.reshape(q.shape)
```
